```python
import os as _os
_os.environ.setdefault("JAX_PLATFORMS", "cpu")
import jax
import jax.numpy as jnp

def _softmax(x, axis=-1):
    return jax.nn.softmax(x, axis=axis)
def _gelu(x):
    return jax.nn.gelu(x, approximate=True)
def _silu(x):
    return jax.nn.silu(x)
def _sigmoid(x):
    return jax.nn.sigmoid(x)
def _layernorm(x, axis=-1, eps=1e-5):
    m = jnp.mean(x, axis=axis, keepdims=True)
    v = jnp.var(x, axis=axis, keepdims=True)
    return (x - m) / jnp.sqrt(v + eps)
def _scatter_add(tgt, idx, src, axis=0):
    return tgt.at[idx].add(src)
def _segment_sum(src, seg, n):
    return jax.ops.segment_sum(src, seg, n)
class _Rng:
    def __init__(self, key):
        self._k = key
    def _next(self):
        self._k, sub = jax.random.split(self._k)
        return sub
    def normal(self, shape):
        return jax.random.normal(self._next(), shape, dtype=jnp.bfloat16)
    def randint(self, lo, hi, shape):
        return jax.random.randint(self._next(), shape, lo, hi, dtype=jnp.int32)
    def uniform(self, shape, lo=0.0, hi=1.0):
        return jax.random.uniform(self._next(), shape, jnp.bfloat16, lo, hi)
    def permutation(self, n):
        return jax.random.permutation(self._next(), n)


kernel_name = 'concat_heads__mha_block_cached__mha_block_cached__near_ridge'

def setup_inputs():
    _rng = _Rng(jax.random.key(int.from_bytes(__import__("os").urandom(4), "little")))
    _w = (lambda a: (lambda t: t.astype(jnp.bfloat16) if jnp.issubdtype(t.dtype, jnp.floating) else t)(jnp.asarray(a)))
    def _A_setup():
        B, Sq, D = 8, 160, 512
        H, Sk, Dh = 32, 512, 128
        return {
            "x": _w((lambda *s: _rng.normal(s) * 0.8)(B, Sq, D)),
            "k_cache": _w((lambda *s: _rng.normal(s) * 0.8)(B, H, Sk, Dh)),
            "v_cache": _w((lambda *s: _rng.normal(s) * 0.05)(B, H, Sk, Dh)),
            "wq": _w((lambda *s: _rng.normal(s) * 0.8)(D, H * Dh) * (D ** -0.5)),
            "wo": _w((lambda *s: _rng.normal(s) * 0.05)(H * Dh, D) * ((H * Dh) ** -0.5)),
        }
    _A_in = _A_setup()

    def _B_setup():
        B, Sq, D = 8, 160, 512
        H, Sk, Dh = 32, 512, 128
        return {
            "x": _w((lambda *s: _rng.normal(s) * 0.8)(B, Sq, D)),
            "k_cache": _w((lambda *s: _rng.normal(s) * 0.8)(B, H, Sk, Dh)),
            "v_cache": _w((lambda *s: _rng.normal(s) * 0.05)(B, H, Sk, Dh)),
            "wq": _w((lambda *s: _rng.normal(s) * 0.8)(D, H * Dh) * (D ** -0.5)),
            "wo": _w((lambda *s: _rng.normal(s) * 0.05)(H * Dh, D) * ((H * Dh) ** -0.5)),
        }
    _B_in = _B_setup()

    return {
        "A_x": _A_in["x"],
        "A_k_cache": _A_in["k_cache"],
        "A_v_cache": _A_in["v_cache"],
        "A_wq": _A_in["wq"],
        "A_wo": _A_in["wo"],
        "B_x": _B_in["x"],
        "B_k_cache": _B_in["k_cache"],
        "B_v_cache": _B_in["v_cache"],
        "B_wq": _B_in["wq"],
        "B_wo": _B_in["wo"],
    }

def reference(A_x, A_k_cache, A_v_cache, A_wq, A_wo, B_x, B_k_cache, B_v_cache, B_wq, B_wo):
    def _A_ref(x, k_cache, v_cache, wq, wo):
        B, Sq, D = x.shape
        H, Dh = 32, 128
        q = (lambda x, *d: x.transpose(*d))((x @ wq).reshape(B, Sq, H, Dh), 0, 2, 1, 3)
        scores = jnp.einsum("bhqd,bhkd->bhqk", q, k_cache) * (Dh ** -0.5)
        p = _softmax(scores, axis=-1)
        o = jnp.einsum("bhqk,bhkd->bhqd", p, v_cache)
        return (lambda x, *d: x.transpose(*d))(o, 0, 2, 1, 3).reshape(B, Sq, H * Dh) @ wo

    def _B_ref(x, k_cache, v_cache, wq, wo):
        B, Sq, D = x.shape
        H, Dh = 32, 128
        q = (lambda x, *d: x.transpose(*d))((x @ wq).reshape(B, Sq, H, Dh), 0, 2, 1, 3)
        scores = jnp.einsum("bhqd,bhkd->bhqk", q, k_cache) * (Dh ** -0.5)
        p = _softmax(scores, axis=-1)
        o = jnp.einsum("bhqk,bhkd->bhqd", p, v_cache)
        return (lambda x, *d: x.transpose(*d))(o, 0, 2, 1, 3).reshape(B, Sq, H * Dh) @ wo

    a = _A_ref(A_x, A_k_cache, A_v_cache, A_wq, A_wo)
    b = _B_ref(B_x, B_k_cache, B_v_cache, B_wq, B_wo)
    return jnp.concatenate([a, b], axis=-1)
```

```python
import jax
import jax.numpy as jnp
from jax import lax
import jax.experimental.pallas as pl
import jax.experimental.pallas.tpu as pltpu

B, SQ, D = 8, 160, 512
H, SK, DH = 32, 512, 128
M = B * SQ
LOG2E = 1.4426950408889634
HB = int(4)
NBUF = int(3)
L = int(5)
XC = int(4)
OC = int(8)
PH = int(2)
SCOPES = int(0)
NG = H // HB
T = 2 * NG
GW = HB * DH
RQ = L + 1
NP = (L * HB) // PH
assert 1 <= L <= NG and NBUF - 1 <= NG - L and (L * HB) % PH == 0 and HB % PH == 0


def _scope(name):
    import contextlib
    return jax.named_scope(name) if SCOPES else contextlib.nullcontext()


def _qk(qb, k):
    return lax.dot_general(qb, k, (((1,), (1,)), ((), ())), preferred_element_type=jnp.float32)


def _softmax_pv(s, v):
    m = jnp.max(s, axis=-1, keepdims=True)
    p = jnp.exp2(s - m)
    l = jnp.sum(p, axis=-1, keepdims=True)
    o = jnp.dot(p.astype(jnp.bfloat16), v, preferred_element_type=jnp.float32)
    return (o * pl.reciprocal(l, approx=True)).astype(jnp.bfloat16)


def _inc(i, n):
    return jnp.where(i + 1 == n, 0, i + 1)


def kernel(xa, ka, va, wqa, woa, xb, kb, vb, wqb, wob, out_hbm,
           x_buf, k_buf, v_buf, wq_buf, wo_buf, wq0_buf, q_buf, acc, o_buf, sems, wq0_sem, xsem, osem):
    srcs = ((xa, ka, va, wqa, woa), (xb, kb, vb, wqb, wob))

    def kv_copies(br, grp, slot):
        _, k_hbm, v_hbm, _, wo_hbm = srcs[br]
        c0 = pl.multiple_of(grp * GW, GW)
        h0 = grp * HB
        return [
            pltpu.make_async_copy(k_hbm.at[:, pl.ds(h0, HB)], k_buf.at[slot], sems.at[slot, 0]),
            pltpu.make_async_copy(v_hbm.at[:, pl.ds(h0, HB)], v_buf.at[slot], sems.at[slot, 1]),
            pltpu.make_async_copy(wo_hbm.at[pl.ds(c0, GW), :], wo_buf.at[slot], sems.at[slot, 2]),
        ]

    def wq_copy(br, grp, slot):
        c0 = pl.multiple_of(grp * GW, GW)
        return pltpu.make_async_copy(srcs[br][3].at[:, pl.ds(c0, GW)], wq_buf.at[slot], sems.at[slot, 3])

    def wq0_copy(p):
        c0 = p * PH * DH if isinstance(p, int) else pl.multiple_of(p * PH * DH, PH * DH)
        return pltpu.make_async_copy(wqa.at[:, pl.ds(c0, PH * DH)], wq0_buf.at[p], wq0_sem.at[p])

    XR = M // XC

    def xa_copy(c):
        r0 = c * XR if isinstance(c, int) else pl.multiple_of(c * XR, XR)
        return pltpu.make_async_copy(xa.at[pl.ds(r0, XR)], x_buf.at[0, pl.ds(r0, XR)], xsem.at[c])

    def xb_copy():
        return pltpu.make_async_copy(xb, x_buf.at[1], xsem.at[XC])

    def outa_copy():
        return pltpu.make_async_copy(o_buf.at[0], out_hbm.at[:, 0:D], osem.at[OC])

    OR = M // OC

    def outb_copy(c):
        return pltpu.make_async_copy(o_buf.at[1, pl.ds(c * OR, OR)], out_hbm.at[pl.ds(c * OR, OR), D:2 * D], osem.at[c])

    def qscale(q):
        return (q * (DH ** -0.5 * LOG2E)).astype(jnp.bfloat16)

    def qproj(br, wq_ref, qslot):
        for hh in range(HB):
            q = jnp.dot(x_buf[br], wq_ref[:, hh * DH:(hh + 1) * DH], preferred_element_type=jnp.float32)
            q_buf[qslot, :, hh * DH:(hh + 1) * DH] = qscale(q)

    def attn_op(br, slot, qslot, hook, out_hook=None):
        units = [(hh, b) for hh in range(HB) for b in range(B)]

        def qk(u):
            hh, b = u
            return _qk(q_buf[qslot, b * SQ:(b + 1) * SQ, hh * DH:(hh + 1) * DH], k_buf[slot, b, hh])

        outs = {}
        s_next = qk(units[0])
        for i, (hh, b) in enumerate(units):
            s_cur = s_next
            if i + 1 < len(units):
                s_next = qk(units[i + 1])
            outs[hh, b] = _softmax_pv(s_cur, v_buf[slot, b, hh])
            if i == 0:
                hook()
        o = jnp.concatenate(
            [jnp.concatenate([outs[hh, b] for b in range(B)], axis=0) for hh in range(HB)], axis=1)
        if out_hook is None:
            new = acc[br] + jnp.dot(o, wo_buf[slot], preferred_element_type=jnp.float32)
            acc[br] = new
            o_buf[br] = new.astype(jnp.bfloat16)
        else:
            r = jnp.dot(o, wo_buf[slot], preferred_element_type=jnp.float32)
            for c in range(OC):
                rows = slice(c * OR, (c + 1) * OR)
                new = acc[br, rows] + r[rows]
                acc[br, rows] = new
                o_buf[br, rows] = new.astype(jnp.bfloat16)
                out_hook(c)

    def issue(lo, hi, fn):
        def body(i, c):
            fn(i)
            return c
        lax.fori_loop(lo, hi, body, 0)

    wq0_copy(0).start()
    issue(0, XC, lambda c: xa_copy(c).start())
    if NP > 1:
        issue(1, NP, lambda p: wq0_copy(p).start())

    def first_groups(g):
        for c in kv_copies(0, g, g):
            c.start()
        wq_copy(0, g + L, g).start()

    issue(0, NBUF - 1, first_groups)
    with _scope("zero"):
        acc[...] = jnp.zeros_like(acc)

    def q_slot_cols(p):
        return (p * PH) // HB, ((p * PH) % HB) * DH

    with _scope("pro0"):
        wq0_copy(0).wait()
        for c in range(XC):
            xa_copy(c).wait()
            rows = pl.ds(c * XR, XR)
            for hh in range(PH):
                q = jnp.dot(x_buf[0, rows], wq0_buf[0, :, hh * DH:(hh + 1) * DH], preferred_element_type=jnp.float32)
                q_buf[0, rows, hh * DH:(hh + 1) * DH] = qscale(q)

    def pro_body(p, carry):
        with _scope("pro"):
            wq0_copy(p).wait()
            g = (p * PH) // HB
            c0 = pl.multiple_of(((p * PH) % HB) * DH, DH)
            for hh in range(PH):
                q = jnp.dot(x_buf[0], wq0_buf[p, :, hh * DH:(hh + 1) * DH], preferred_element_type=jnp.float32)
                q_buf[g, :, pl.ds(c0 + hh * DH, DH)] = qscale(q)
        return carry

    if NP > 1:
        lax.fori_loop(1, NP, pro_body, 0)

    def header(g, slot, with_wq):
        with _scope("wait"):
            for c in kv_copies(0, 0, slot):
                c.wait()
            if with_wq:
                wq_copy(0, 0, slot).wait()

                @pl.when(g == NG - L)
                def _():
                    xb_copy().wait()

    def prefetch(g, nslot, with_wq):
        nxt = g + (NBUF - 1)

        @pl.when(nxt < NG)
        def _():
            for c in kv_copies(0, nxt, nslot):
                c.start()

        @pl.when(jnp.logical_and(nxt >= NG, nxt < T))
        def _():
            for c in kv_copies(1, nxt - NG, nslot):
                c.start()

        if with_wq:
            @pl.when(nxt + L < NG)
            def _():
                wq_copy(0, nxt + L, nslot).start()

            @pl.when(jnp.logical_and(nxt + L >= NG, nxt + L < T))
            def _():
                wq_copy(1, nxt + L - NG, nslot).start()

            @pl.when(g == 0)
            def _():
                xb_copy().start()

            @pl.when(g == NG)
            def _():
                outa_copy().start()

    def main_body(g, carry):
        slot, nslot, qr, qw = carry
        with _scope("main"):
            header(g, slot, True)
            br = g // NG
            brq = (g + L) // NG
            attn_op(br, slot, qr, lambda: prefetch(g, nslot, True))
            qproj(brq, wq_buf.at[slot], qw)
        return _inc(slot, NBUF), _inc(nslot, NBUF), _inc(qr, RQ), _inc(qw, RQ)

    def tail_body(g, carry):
        slot, nslot, qr, qw = carry

        def out_hook(c):
            @pl.when(g == T - 1)
            def _():
                outb_copy(c).start()

        with _scope("tail"):
            header(g, slot, False)
            attn_op(1, slot, qr, lambda: prefetch(g, nslot, False), out_hook)
        return _inc(slot, NBUF), _inc(nslot, NBUF), _inc(qr, RQ), _inc(qw, RQ)

    z = jnp.int32(0)
    carry = (z, z + (NBUF - 1), z, z + L)
    carry = lax.fori_loop(0, T - L, main_body, carry)
    lax.fori_loop(T - L, T, tail_body, carry)
    with _scope("epi"):
        outa_copy().wait()
        for c in range(OC):
            outb_copy(c).wait()


@jax.jit
def pallas_concat_heads__mha_block_cached__mha_block_cached__near_ridge_kernel(
        A_x, A_k_cache, A_v_cache, A_wq, A_wo, B_x, B_k_cache, B_v_cache, B_wq, B_wo):
    any_spec = pl.BlockSpec(memory_space=pl.ANY)
    out = pl.pallas_call(
        kernel,
        in_specs=[any_spec] * 10,
        out_specs=any_spec,
        out_shape=jax.ShapeDtypeStruct((M, 2 * D), jnp.bfloat16),
        scratch_shapes=[
            pltpu.VMEM((2, M, D), jnp.bfloat16),
            pltpu.VMEM((NBUF, B, HB, SK, DH), jnp.bfloat16),
            pltpu.VMEM((NBUF, B, HB, SK, DH), jnp.bfloat16),
            pltpu.VMEM((NBUF, D, GW), jnp.bfloat16),
            pltpu.VMEM((NBUF, GW, D), jnp.bfloat16),
            pltpu.VMEM((NP, D, PH * DH), jnp.bfloat16),
            pltpu.VMEM((RQ, M, GW), jnp.bfloat16),
            pltpu.VMEM((2, M, D), jnp.float32),
            pltpu.VMEM((2, M, D), jnp.bfloat16),
            pltpu.SemaphoreType.DMA((NBUF, 4)),
            pltpu.SemaphoreType.DMA((NP,)),
            pltpu.SemaphoreType.DMA((XC + 1,)),
            pltpu.SemaphoreType.DMA((OC + 1,)),
        ],
        compiler_params=pltpu.CompilerParams(vmem_limit_bytes=110 * 1024 * 1024,
                                             disable_bounds_checks=True),
    )(A_x.reshape(M, D), A_k_cache, A_v_cache, A_wq, A_wo,
      B_x.reshape(M, D), B_k_cache, B_v_cache, B_wq, B_wo)
    return out.reshape(B, SQ, 2 * D)
```

```python
import jax
import jax.numpy as jnp
from jax import lax
import jax.experimental.pallas as pl
import jax.experimental.pallas.tpu as pltpu

B, SQ, D = 8, 160, 512
H, SK, DH = 32, 512, 128
M = B * SQ

HB = 4
NBUF = 3
L = 5
NG = H // HB
T = 2 * NG
GW = HB * DH
RQ = L + 1

X_CHUNKS = (336, 432, 512)
Q0_HEADS = 2
Q_PASSES = (4, 14)
OUT_CHUNKS = (256, 256, 256, 256, 128, 64, 32, 32)

assert Q0_HEADS + sum(Q_PASSES) == L * HB and sum(X_CHUNKS) == M and sum(OUT_CHUNKS) == M
assert NBUF - 1 <= NG - L

Q_SCALE = DH ** -0.5 * 1.4426950408889634


def _offsets(sizes):
    return [sum(sizes[:i]) for i in range(len(sizes))]


X_OFF, OUT_OFF = _offsets(X_CHUNKS), _offsets(OUT_CHUNKS)
WQ0_HEAD0 = [0] + [Q0_HEADS + o for o in _offsets(Q_PASSES)]
WQ0_NHEADS = [Q0_HEADS] + list(Q_PASSES)


def _dot(a, b):
    return jnp.dot(a, b, preferred_element_type=jnp.float32)


def _dot_nt(a, b):
    return lax.dot_general(a, b, (((1,), (1,)), ((), ())), preferred_element_type=jnp.float32)


def _softmax_pv(s, v):
    m = jnp.max(s, axis=-1, keepdims=True)
    p = jnp.exp2(s - m)
    l = jnp.sum(p, axis=-1, keepdims=True)
    r = pl.reciprocal(l, approx=True)
    r = r * (2.0 - l * r)
    return (_dot(p.astype(jnp.bfloat16), v) * r).astype(jnp.bfloat16)


def _next(i, n):
    return jnp.where(i + 1 == n, 0, i + 1)


def _kernel(xa, ka, va, wqa, woa, xb, kb, vb, wqb, wob, out_hbm,
            x_buf, k_buf, v_buf, wq_buf, wo_buf, wq0_buf, acc, o_buf,
            ring_sem, wq0_sem, x_sem, out_sem, *q_bufs):
    srcs = ((xa, ka, va, wqa, woa), (xb, kb, vb, wqb, wob))

    def ring_copy(kind, br, grp, slot):
        _, k_hbm, v_hbm, _, wo_hbm = srcs[br]
        if kind == 2:
            rows = pl.ds(pl.multiple_of(grp * GW, GW), GW)
            return pltpu.make_async_copy(wo_hbm.at[rows, :], wo_buf.at[slot], ring_sem.at[slot, 2])
        src, dst = ((k_hbm, k_buf), (v_hbm, v_buf))[kind]
        return pltpu.make_async_copy(src.at[:, pl.ds(grp * HB, HB)], dst.at[slot], ring_sem.at[slot, kind])

    def ring_start(br, grp, slot):
        for kind in range(3):
            ring_copy(kind, br, grp, slot).start()

    def wq_copy(br, grp, slot):
        cols = pl.ds(pl.multiple_of(grp * GW, GW), GW)
        return pltpu.make_async_copy(srcs[br][3].at[:, cols], wq_buf.at[slot], ring_sem.at[slot, 3])

    def wq0_copy(p):
        cols = pl.ds(WQ0_HEAD0[p] * DH, WQ0_NHEADS[p] * DH)
        return pltpu.make_async_copy(wqa.at[:, cols], wq0_buf.at[:, cols], wq0_sem.at[p])

    def xa_copy(c):
        rows = pl.ds(X_OFF[c], X_CHUNKS[c])
        return pltpu.make_async_copy(xa.at[rows], x_buf.at[0, rows], x_sem.at[c])

    def xb_copy():
        return pltpu.make_async_copy(xb, x_buf.at[1], x_sem.at[len(X_CHUNKS)])

    def outa_copy():
        return pltpu.make_async_copy(o_buf.at[0], out_hbm.at[:, 0:D], out_sem.at[len(OUT_CHUNKS)])

    def outb_copy(c):
        rows = pl.ds(OUT_OFF[c], OUT_CHUNKS[c])
        return pltpu.make_async_copy(o_buf.at[1, rows], out_hbm.at[rows, D:2 * D], out_sem.at[c])

    def to_q(q):
        return (q * Q_SCALE).astype(jnp.bfloat16)

    def q_proj(br, slot, qslot, heads):
        for hh in heads:
            q_bufs[hh][qslot] = to_q(_dot(x_buf[br], wq_buf[slot, :, hh * DH:(hh + 1) * DH]))

    def attn_out(br, slot, qslot, after_first_unit, out_chunk_done=None):
        units = [(hh, b) for hh in range(HB) for b in range(B)]

        def scores(unit):
            hh, b = unit
            return _dot_nt(q_bufs[hh][qslot, b * SQ:(b + 1) * SQ, :], k_buf[slot, b, hh])

        outs = {}
        s_next = scores(units[0])
        for i, (hh, b) in enumerate(units):
            s_cur = s_next
            if i + 1 < len(units):
                s_next = scores(units[i + 1])
            outs[hh, b] = _softmax_pv(s_cur, v_buf[slot, b, hh])
            if i == 0:
                after_first_unit()
        o = jnp.concatenate(
            [jnp.concatenate([outs[hh, b] for b in range(B)], axis=0) for hh in range(HB)], axis=1)
        if out_chunk_done is None:
            new = acc[br] + _dot(o, wo_buf[slot])
            acc[br] = new
            o_buf[br] = new.astype(jnp.bfloat16)
        else:
            for c in range(len(OUT_CHUNKS)):
                rows = slice(OUT_OFF[c], OUT_OFF[c] + OUT_CHUNKS[c])
                new = acc[br, rows] + _dot(o[rows], wo_buf[slot])
                acc[br, rows] = new
                o_buf[br, rows] = new.astype(jnp.bfloat16)
                out_chunk_done(c)

    def start_in_order(fns):
        def body(i, carry):
            for k, fn in enumerate(fns):
                pl.when(i == k)(fn)
            return carry
        lax.fori_loop(0, len(fns), body, 0)

    first = [lambda: wq0_copy(0).start()]
    first += [lambda c=c: xa_copy(c).start() for c in range(len(X_CHUNKS))]
    first += [lambda p=p: wq0_copy(p).start() for p in range(1, len(WQ0_NHEADS))]
    for g0 in range(NBUF - 1):
        first += [lambda g=g0, k=k: ring_copy(k, 0, g, g).start() for k in range(3)]
        first += [lambda g=g0: wq_copy(0, g + L, g).start()]
    start_in_order(first)

    acc[...] = jnp.zeros_like(acc)

    wq0_copy(0).wait()
    for c in range(len(X_CHUNKS)):
        xa_copy(c).wait()
        rows = pl.ds(X_OFF[c], X_CHUNKS[c])
        for h in range(Q0_HEADS):
            q_bufs[h % HB][h // HB, rows] = to_q(_dot(x_buf[0, rows], wq0_buf[:, h * DH:(h + 1) * DH]))
    for p in range(1, len(WQ0_NHEADS)):
        wq0_copy(p).wait()
        for h in range(WQ0_HEAD0[p], WQ0_HEAD0[p] + WQ0_NHEADS[p]):
            q_bufs[h % HB][h // HB] = to_q(_dot(x_buf[0], wq0_buf[:, h * DH:(h + 1) * DH]))

    def wait_group(g, slot, with_wq):
        for kind in range(3):
            ring_copy(kind, 0, 0, slot).wait()
        if with_wq:
            wq_copy(0, 0, slot).wait()

            @pl.when(g == NG - L)
            def _():
                xb_copy().wait()

    def prefetch(g, nslot, with_wq):
        nxt = g + (NBUF - 1)

        @pl.when(nxt < NG)
        def _():
            ring_start(0, nxt, nslot)

        @pl.when(jnp.logical_and(nxt >= NG, nxt < T))
        def _():
            ring_start(1, nxt - NG, nslot)

        if with_wq:
            @pl.when(nxt + L < NG)
            def _():
                wq_copy(0, nxt + L, nslot).start()

            @pl.when(jnp.logical_and(nxt + L >= NG, nxt + L < T))
            def _():
                wq_copy(1, nxt + L - NG, nslot).start()

            @pl.when(g == 0)
            def _():
                xb_copy().start()

            @pl.when(g == NG)
            def _():
                outa_copy().start()

    def advance(carry):
        slot, nslot, qr, qw = carry
        return _next(slot, NBUF), _next(nslot, NBUF), _next(qr, RQ), _next(qw, RQ)

    def main_body(g, carry):
        slot, nslot, qr, qw = carry
        wait_group(g, slot, True)
        br, brq = g // NG, (g + L) // NG
        q_proj(brq, slot, qw, range(HB - 1, HB))
        attn_out(br, slot, qr, lambda: prefetch(g, nslot, True))
        q_proj(brq, slot, qw, range(0, HB - 1))
        return advance(carry)

    def tail_body(g, carry):
        slot, nslot, qr, _ = carry

        def out_chunk_done(c):
            @pl.when(g == T - 1)
            def _():
                outb_copy(c).start()

        wait_group(g, slot, False)
        attn_out(1, slot, qr, lambda: prefetch(g, nslot, False), out_chunk_done)
        return advance(carry)

    zero = jnp.int32(0)
    carry = lax.fori_loop(0, T - L, main_body, (zero, zero + (NBUF - 1), zero, zero + L))
    lax.fori_loop(T - L, T, tail_body, carry)

    outa_copy().wait()
    for c in range(len(OUT_CHUNKS)):
        outb_copy(c).wait()


@jax.jit
def pallas_concat_heads__mha_block_cached__mha_block_cached__near_ridge_kernel(
    A_x: jax.Array,
    A_k_cache: jax.Array,
    A_v_cache: jax.Array,
    A_wq: jax.Array,
    A_wo: jax.Array,
    B_x: jax.Array,
    B_k_cache: jax.Array,
    B_v_cache: jax.Array,
    B_wq: jax.Array,
    B_wo: jax.Array,
):
    in_hbm = pl.BlockSpec(memory_space=pl.ANY)
    out = pl.pallas_call(
        _kernel,
        in_specs=[in_hbm] * 10,
        out_specs=in_hbm,
        out_shape=jax.ShapeDtypeStruct((M, 2 * D), jnp.bfloat16),
        scratch_shapes=[
            pltpu.VMEM((2, M, D), jnp.bfloat16),
            pltpu.VMEM((NBUF, B, HB, SK, DH), jnp.bfloat16),
            pltpu.VMEM((NBUF, B, HB, SK, DH), jnp.bfloat16),
            pltpu.VMEM((NBUF, D, GW), jnp.bfloat16),
            pltpu.VMEM((NBUF, GW, D), jnp.bfloat16),
            pltpu.VMEM((D, L * GW), jnp.bfloat16),
            pltpu.VMEM((2, M, D), jnp.float32),
            pltpu.VMEM((2, M, D), jnp.bfloat16),
            pltpu.SemaphoreType.DMA((NBUF, 4)),
            pltpu.SemaphoreType.DMA((len(WQ0_NHEADS),)),
            pltpu.SemaphoreType.DMA((len(X_CHUNKS) + 1,)),
            pltpu.SemaphoreType.DMA((len(OUT_CHUNKS) + 1,)),
        ] + [pltpu.VMEM((RQ, M, DH), jnp.bfloat16) for _ in range(HB)],
        compiler_params=pltpu.CompilerParams(
            vmem_limit_bytes=110 * 1024 * 1024,
            disable_bounds_checks=True,
            disable_semaphore_checks=True,
        ),
    )(A_x.reshape(M, D), A_k_cache, A_v_cache, A_wq, A_wo,
      B_x.reshape(M, D), B_k_cache, B_v_cache, B_wq, B_wo)
    return out.reshape(B, SQ, 2 * D)
```

```python
import jax
import jax.numpy as jnp
from jax import lax
import jax.experimental.pallas as pl
import jax.experimental.pallas.tpu as pltpu

B, SQ, D = 8, 160, 512
H, SK, DH = 32, 512, 128
M = B * SQ

HB = 4
NBUF = 3
L = 5
NG = H // HB
T = 2 * NG
GW = HB * DH
RQ = L + 1

X_CHUNKS = (176, 272, 368, 464)
Q0_HEADS = 2
Q_PASSES = (4, 14)
OUT_CHUNKS = (256, 256, 256, 256, 128, 64, 32, 32)

assert Q0_HEADS + sum(Q_PASSES) == L * HB and sum(X_CHUNKS) == M and sum(OUT_CHUNKS) == M
assert NBUF - 1 <= NG - L

Q_SCALE = DH ** -0.5 * 1.4426950408889634


def _offsets(sizes):
    return [sum(sizes[:i]) for i in range(len(sizes))]


X_OFF, OUT_OFF = _offsets(X_CHUNKS), _offsets(OUT_CHUNKS)
WQ0_HEAD0 = [0] + [Q0_HEADS + o for o in _offsets(Q_PASSES)]
WQ0_NHEADS = [Q0_HEADS] + list(Q_PASSES)


def _dot(a, b):
    return jnp.dot(a, b, preferred_element_type=jnp.float32)


def _dot_nt(a, b):
    return lax.dot_general(a, b, (((1,), (1,)), ((), ())), preferred_element_type=jnp.float32)


def _softmax_pv(s, v):
    m = jnp.max(s, axis=-1, keepdims=True)
    p = jnp.exp2(s - m)
    l = jnp.sum(p, axis=-1, keepdims=True)
    r = pl.reciprocal(l, approx=True)
    r = r * (2.0 - l * r)
    return (_dot(p.astype(jnp.bfloat16), v) * r).astype(jnp.bfloat16)


def _next(i, n):
    return jnp.where(i + 1 == n, 0, i + 1)


def _kernel(xa, ka, va, wqa, woa, xb, kb, vb, wqb, wob, out_hbm,
            x_buf, k_buf, v_buf, wq_buf, wo_buf, wq0_buf, acc, o_buf,
            ring_sem, wq0_sem, x_sem, out_sem, *q_bufs):
    srcs = ((xa, ka, va, wqa, woa), (xb, kb, vb, wqb, wob))

    def ring_copy(kind, br, grp, slot):
        _, k_hbm, v_hbm, _, wo_hbm = srcs[br]
        if kind == 2:
            rows = pl.ds(pl.multiple_of(grp * GW, GW), GW)
            return pltpu.make_async_copy(wo_hbm.at[rows, :], wo_buf.at[slot], ring_sem.at[slot, 2])
        src, dst = ((k_hbm, k_buf), (v_hbm, v_buf))[kind]
        return pltpu.make_async_copy(src.at[:, pl.ds(grp * HB, HB)], dst.at[slot], ring_sem.at[slot, kind])

    def ring_start(br, grp, slot):
        for kind in range(3):
            ring_copy(kind, br, grp, slot).start()

    def wq_copy(br, grp, slot):
        cols = pl.ds(pl.multiple_of(grp * GW, GW), GW)
        return pltpu.make_async_copy(srcs[br][3].at[:, cols], wq_buf.at[slot], ring_sem.at[slot, 3])

    def wq0_copy(p):
        cols = pl.ds(WQ0_HEAD0[p] * DH, WQ0_NHEADS[p] * DH)
        return pltpu.make_async_copy(wqa.at[:, cols], wq0_buf.at[:, cols], wq0_sem.at[p])

    def xa_copy(c):
        rows = pl.ds(X_OFF[c], X_CHUNKS[c])
        return pltpu.make_async_copy(xa.at[rows], x_buf.at[0, rows], x_sem.at[c])

    def xb_copy():
        return pltpu.make_async_copy(xb, x_buf.at[1], x_sem.at[len(X_CHUNKS)])

    def outa_copy():
        return pltpu.make_async_copy(o_buf.at[0], out_hbm.at[:, 0:D], out_sem.at[len(OUT_CHUNKS)])

    def outb_copy(c):
        rows = pl.ds(OUT_OFF[c], OUT_CHUNKS[c])
        return pltpu.make_async_copy(o_buf.at[1, rows], out_hbm.at[rows, D:2 * D], out_sem.at[c])

    def to_q(q):
        return (q * Q_SCALE).astype(jnp.bfloat16)

    def q_proj(br, slot, qslot, heads):
        for hh in heads:
            q_bufs[hh][qslot] = to_q(_dot(x_buf[br], wq_buf[slot, :, hh * DH:(hh + 1) * DH]))

    def attn_out(br, slot, qslot, after_first_unit, out_chunk_done=None):
        units = [(hh, b) for hh in range(HB) for b in range(B)]

        def scores(unit):
            hh, b = unit
            return _dot_nt(q_bufs[hh][qslot, b * SQ:(b + 1) * SQ, :], k_buf[slot, b, hh])

        outs = {}
        s_next = scores(units[0])
        for i, (hh, b) in enumerate(units):
            s_cur = s_next
            if i + 1 < len(units):
                s_next = scores(units[i + 1])
            outs[hh, b] = _softmax_pv(s_cur, v_buf[slot, b, hh])
            if i == 0:
                after_first_unit()
        o = jnp.concatenate(
            [jnp.concatenate([outs[hh, b] for b in range(B)], axis=0) for hh in range(HB)], axis=1)
        if out_chunk_done is None:
            new = acc[br] + _dot(o, wo_buf[slot])
            acc[br] = new
            o_buf[br] = new.astype(jnp.bfloat16)
        else:
            for c in range(len(OUT_CHUNKS)):
                rows = slice(OUT_OFF[c], OUT_OFF[c] + OUT_CHUNKS[c])
                new = acc[br, rows] + _dot(o[rows], wo_buf[slot])
                acc[br, rows] = new
                o_buf[br, rows] = new.astype(jnp.bfloat16)
                out_chunk_done(c)

    def start_in_order(fns):
        def body(i, carry):
            for k, fn in enumerate(fns):
                pl.when(i == k)(fn)
            return carry
        lax.fori_loop(0, len(fns), body, 0)

    start_in_order([lambda: wq0_copy(0).start()] + [lambda c=c: xa_copy(c).start() for c in range(len(X_CHUNKS))])
    start_in_order([lambda p=p: wq0_copy(p).start() for p in range(1, len(WQ0_NHEADS))])

    def start_group(g0, carry):
        ring_start(0, g0, g0)
        wq_copy(0, g0 + L, g0).start()
        return carry
    lax.fori_loop(0, NBUF - 1, start_group, 0)

    acc[...] = jnp.zeros_like(acc)

    wq0_copy(0).wait()
    for c in range(len(X_CHUNKS)):
        xa_copy(c).wait()
        rows = pl.ds(X_OFF[c], X_CHUNKS[c])
        for h in range(Q0_HEADS):
            q_bufs[h % HB][h // HB, rows] = to_q(_dot(x_buf[0, rows], wq0_buf[:, h * DH:(h + 1) * DH]))
    for p in range(1, len(WQ0_NHEADS)):
        wq0_copy(p).wait()
        for h in range(WQ0_HEAD0[p], WQ0_HEAD0[p] + WQ0_NHEADS[p]):
            q_bufs[h % HB][h // HB] = to_q(_dot(x_buf[0], wq0_buf[:, h * DH:(h + 1) * DH]))

    def wait_group(g, slot, with_wq):
        for kind in range(3):
            ring_copy(kind, 0, 0, slot).wait()
        if with_wq:
            wq_copy(0, 0, slot).wait()

            @pl.when(g == NG - L)
            def _():
                xb_copy().wait()

    def prefetch(g, nslot, with_wq):
        nxt = g + (NBUF - 1)

        @pl.when(nxt < NG)
        def _():
            ring_start(0, nxt, nslot)

        @pl.when(jnp.logical_and(nxt >= NG, nxt < T))
        def _():
            ring_start(1, nxt - NG, nslot)

        if with_wq:
            @pl.when(nxt + L < NG)
            def _():
                wq_copy(0, nxt + L, nslot).start()

            @pl.when(jnp.logical_and(nxt + L >= NG, nxt + L < T))
            def _():
                wq_copy(1, nxt + L - NG, nslot).start()

            @pl.when(g == 0)
            def _():
                xb_copy().start()

            @pl.when(g == NG)
            def _():
                outa_copy().start()

    def advance(carry):
        slot, nslot, qr, qw = carry
        return _next(slot, NBUF), _next(nslot, NBUF), _next(qr, RQ), _next(qw, RQ)

    def main_body(g, carry):
        slot, nslot, qr, qw = carry
        wait_group(g, slot, True)
        br, brq = g // NG, (g + L) // NG
        q_proj(brq, slot, qw, range(HB - 1, HB))
        attn_out(br, slot, qr, lambda: prefetch(g, nslot, True))
        q_proj(brq, slot, qw, range(0, HB - 1))
        return advance(carry)

    def tail_body(g, carry):
        slot, nslot, qr, _ = carry

        def out_chunk_done(c):
            @pl.when(g == T - 1)
            def _():
                outb_copy(c).start()

        wait_group(g, slot, False)
        attn_out(1, slot, qr, lambda: prefetch(g, nslot, False), out_chunk_done)
        return advance(carry)

    zero = jnp.int32(0)
    carry = lax.fori_loop(0, T - L, main_body, (zero, zero + (NBUF - 1), zero, zero + L))
    lax.fori_loop(T - L, T, tail_body, carry)

    outa_copy().wait()
    for c in range(len(OUT_CHUNKS)):
        outb_copy(c).wait()


@jax.jit
def pallas_concat_heads__mha_block_cached__mha_block_cached__near_ridge_kernel(
    A_x: jax.Array,
    A_k_cache: jax.Array,
    A_v_cache: jax.Array,
    A_wq: jax.Array,
    A_wo: jax.Array,
    B_x: jax.Array,
    B_k_cache: jax.Array,
    B_v_cache: jax.Array,
    B_wq: jax.Array,
    B_wo: jax.Array,
):
    in_hbm = pl.BlockSpec(memory_space=pl.ANY)
    out = pl.pallas_call(
        _kernel,
        in_specs=[in_hbm] * 10,
        out_specs=in_hbm,
        out_shape=jax.ShapeDtypeStruct((M, 2 * D), jnp.bfloat16),
        scratch_shapes=[
            pltpu.VMEM((2, M, D), jnp.bfloat16),
            pltpu.VMEM((NBUF, B, HB, SK, DH), jnp.bfloat16),
            pltpu.VMEM((NBUF, B, HB, SK, DH), jnp.bfloat16),
            pltpu.VMEM((NBUF, D, GW), jnp.bfloat16),
            pltpu.VMEM((NBUF, GW, D), jnp.bfloat16),
            pltpu.VMEM((D, L * GW), jnp.bfloat16),
            pltpu.VMEM((2, M, D), jnp.float32),
            pltpu.VMEM((2, M, D), jnp.bfloat16),
            pltpu.SemaphoreType.DMA((NBUF, 4)),
            pltpu.SemaphoreType.DMA((len(WQ0_NHEADS),)),
            pltpu.SemaphoreType.DMA((len(X_CHUNKS) + 1,)),
            pltpu.SemaphoreType.DMA((len(OUT_CHUNKS) + 1,)),
        ] + [pltpu.VMEM((RQ, M, DH), jnp.bfloat16) for _ in range(HB)],
        compiler_params=pltpu.CompilerParams(
            vmem_limit_bytes=110 * 1024 * 1024,
            disable_bounds_checks=True,
            disable_semaphore_checks=True,
        ),
    )(A_x.reshape(M, D), A_k_cache, A_v_cache, A_wq, A_wo,
      B_x.reshape(M, D), B_k_cache, B_v_cache, B_wq, B_wo)
    return out.reshape(B, SQ, 2 * D)
```
